```python
import jax
import jax.numpy as jnp

def _softmax(x, axis=-1):
    return jax.nn.softmax(x, axis=axis)
def _gelu(x):
    return jax.nn.gelu(x, approximate=True)
def _silu(x):
    return jax.nn.silu(x)
def _sigmoid(x):
    return jax.nn.sigmoid(x)
def _layernorm(x, axis=-1, eps=1e-5):
    m = jnp.mean(x, axis=axis, keepdims=True)
    v = jnp.var(x, axis=axis, keepdims=True)
    return (x - m) / jnp.sqrt(v + eps)
def _scatter_add(tgt, idx, src, axis=0):
    return tgt.at[idx].add(src)
def _segment_sum(src, seg, n):
    return jax.ops.segment_sum(src, seg, n)
class _Rng:
    def __init__(self, key):
        self._k = key
    def _next(self):
        self._k, sub = jax.random.split(self._k)
        return sub
    def normal(self, shape):
        return jax.random.normal(self._next(), shape, dtype=jnp.bfloat16)
    def randint(self, lo, hi, shape):
        return jax.random.randint(self._next(), shape, lo, hi, dtype=jnp.int32)
    def uniform(self, shape, lo=0.0, hi=1.0):
        return jax.random.uniform(self._next(), shape, jnp.bfloat16, lo, hi)
    def permutation(self, n):
        return jax.random.permutation(self._next(), n)


kernel_name = 'sequential_preLN__linear_attn_block__moe_arch_mod__prompt'

def setup_inputs():
    _rng = _Rng(jax.random.key(int.from_bytes(__import__("os").urandom(4), "little")))
    _w = (lambda a: (lambda t: t.astype(jnp.bfloat16) if jnp.issubdtype(t.dtype, jnp.floating) else t)(jnp.asarray(a)))
    def _A_setup():
        B, S, D = 1, 2048, 1024
        return {
            "x": _w((lambda *s: _rng.normal(s) * 0.05)(B, S, D)),
            "wqkv": _w((lambda *s: _rng.normal(s) * 0.05)(D, 3 * D)),
            "wo": _w((lambda *s: _rng.normal(s) * 0.05)(D, D)),
        }
    _A_in = _A_setup()

    def _B_setup():
        B, S, D, F, C = 1, 2048, 1024, 3584, 2
        return {
            "x": _w((lambda *s: _rng.normal(s) * 0.05)(B, S, D)),
            "w_r": _w((lambda *s: _rng.normal(s) * 0.05)(D)),
            "w_gate": _w((lambda *s: _rng.normal(s) * 0.05)(D, F)),
            "w_up": _w((lambda *s: _rng.normal(s) * 0.05)(D, F)),
            "w_down": _w((lambda *s: _rng.normal(s) * 0.05)(F, D)),
        }
    _B_in = _B_setup()

    return {
        "A_x": _A_in["x"],
        "A_wqkv": _A_in["wqkv"],
        "A_wo": _A_in["wo"],
        "B_x": _B_in["x"],
        "B_w_r": _B_in["w_r"],
        "B_w_gate": _B_in["w_gate"],
        "B_w_up": _B_in["w_up"],
        "B_w_down": _B_in["w_down"],
    }

def reference(A_x, A_wqkv, A_wo, B_x, B_w_r, B_w_gate, B_w_up, B_w_down):
    def _A_ref(x, wqkv, wo):
        B, S, D = x.shape
        H = 32; Dh = D // H
        qkv = (lambda x, *d: x.transpose(*d))((x @ wqkv).reshape(B, S, 3, H, Dh), 2, 0, 3, 1, 4)
        q, k, v = qkv[0], qkv[1], qkv[2]
        phi = lambda t: jnp.where(t > 0, t + 1, jnp.exp(t)) + 1e-6
        pq, pk = phi(q), phi(k)
        kv = jnp.einsum("bhsd,bhse->bhde", pk, v)
        z = jnp.einsum("bhsd->bhd", pk)
        num = jnp.einsum("bhqd,bhde->bhqe", pq, kv)
        den = jnp.einsum("bhqd,bhd->bhq", pq, z)[..., None] + 1e-6
        o = num / den
        return (lambda x, *d: x.transpose(*d))(o, 0, 2, 1, 3).reshape(B, S, D) @ wo

    def _B_ref(x, w_r, w_gate, w_up, w_down):
        B, S, D = x.shape
        C = 2
        r = x @ w_r
        idx = jnp.argsort(-r, axis=-1)[:, :C]
        idx_e = jnp.repeat(idx.reshape(B, C, 1), D, axis=2)
        x_sel = jnp.take_along_axis(x, idx_e, axis=1)
        g = _silu(x_sel @ w_gate)
        u = x_sel @ w_up
        y = (g * u) @ w_down
        r_sel = _sigmoid(jnp.take_along_axis(r, idx, axis=1))
        y = y * r_sel.reshape(B, C, 1)
        b_off = (jnp.arange(B) * S).reshape(B, 1)
        flat_idx = (idx + b_off).reshape(B * C)
        zero = (x * 0.0).reshape(B * S, D)
        upd = _scatter_add(zero, flat_idx, y.reshape(B * C, D), axis=0)
        return x + upd.reshape(B, S, D)

    x = A_x
    h = x + _A_ref(_layernorm(x, axis=-1), A_wqkv, A_wo)
    h2 = h + _B_ref(_layernorm(h, axis=-1), B_w_r, B_w_gate, B_w_up, B_w_down)
    return h2
```

```python
import functools
import jax
import jax.numpy as jnp
from jax import lax
import jax.experimental.pallas as pl
import jax.experimental.pallas.tpu as pltpu

S, D, F, H, DH = 2048, 1024, 3584, 32, 32
TM = 512
NB = S // TM
G = D // 128
BF = jnp.bfloat16
F32 = jnp.float32
NT = (((1,), (1,)), ((), ()))


def _phi(t):
    return jnp.where(t > 0, t + 1.0, jnp.exp(t)) + 1e-6


def _ln(x):
    m = jnp.mean(x, axis=-1, keepdims=True)
    c = x - m
    v = jnp.mean(c * c, axis=-1, keepdims=True)
    return c * lax.rsqrt(v + 1e-5)


def _kernel(x_hbm, wqkv_hbm, wo_hbm, wr_ref, wg_hbm, wu_hbm, wd_hbm, out_hbm,
            x_v, xn_v, pq_v, wq_v, wk_v, wv_v, wkT_v, wo_v, m_v, zb_v, p_acc, z_acc,
            r_v, wg_v, wu_v, wd_v, xsem, wsem, osem):
    def x_copy(i):
        return pltpu.make_async_copy(x_hbm.at[pl.ds(i * TM, TM)], x_v.at[pl.ds(i * TM, TM)], xsem.at[i])

    def o_copy(i):
        return pltpu.make_async_copy(x_v.at[pl.ds(i * TM, TM)], out_hbm.at[pl.ds(i * TM, TM)], osem.at[i])

    cq = pltpu.make_async_copy(wqkv_hbm.at[:, pl.ds(0, D)], wq_v, wsem.at[0])
    ck = pltpu.make_async_copy(wqkv_hbm.at[:, pl.ds(D, D)], wk_v, wsem.at[1])
    cv = pltpu.make_async_copy(wqkv_hbm.at[:, pl.ds(2 * D, D)], wv_v, wsem.at[2])
    co = pltpu.make_async_copy(wo_hbm, wo_v, wsem.at[3])
    cg = pltpu.make_async_copy(wg_hbm, wg_v, wsem.at[4])
    cu = pltpu.make_async_copy(wu_hbm, wu_v, wsem.at[5])
    cd = pltpu.make_async_copy(wd_hbm, wd_v, wsem.at[6])

    x_copy(0).start()
    cq.start()
    for i in range(1, NB):
        x_copy(i).start()
    ck.start()
    cv.start()
    co.start()
    cg.start()
    cu.start()
    cd.start()

    cq.wait()

    with jax.named_scope("phaseA1"):
        @pl.loop(0, NB)
        def _(i):
            x_copy(i).wait()
            rows = pl.ds(pl.multiple_of(i * TM, TM), TM)
            xn = _ln(x_v[rows, :].astype(F32)).astype(BF)
            xn_v[rows, :] = xn
            q = jnp.dot(xn, wq_v[...], preferred_element_type=F32)
            pq_v[rows, :] = _phi(q).astype(BF)

    with jax.named_scope("wkT"):
        ck.wait()
        for g in range(G):
            wkT_v[pl.ds(g * 128, 128), :] = wk_v[:, pl.ds(g * 128, 128)].T
        p_acc[...] = jnp.zeros_like(p_acc)
        z_acc[...] = jnp.zeros_like(z_acc)

    with jax.named_scope("phaseA2"):
        @pl.loop(0, NB)
        def _(i):
            rows = pl.ds(pl.multiple_of(i * TM, TM), TM)
            xn = xn_v[rows, :]
            kT = lax.dot_general(wkT_v[...], xn, NT, preferred_element_type=F32)
            pk = _phi(kT)
            zs = pk[:, 0:128]
            for j in range(1, TM // 128):
                zs = zs + pk[:, j * 128:(j + 1) * 128]
            z_acc[...] += zs
            p_acc[...] += jnp.dot(pk.astype(BF), xn, preferred_element_type=F32)

    with jax.named_scope("mid"):
        cv.wait()
        co.wait()
        rr = lax.broadcasted_iota(jnp.int32, (128, 128), 0) // DH
        cc = lax.broadcasted_iota(jnp.int32, (128, 128), 1) // DH
        mask = rr == cc
        for g in range(G):
            sl = pl.ds(g * 128, 128)
            kv = jnp.dot(p_acc[sl, :].astype(BF), wv_v[:, sl], preferred_element_type=F32)
            kvb = jnp.where(mask, kv, 0.0).astype(BF)
            m_v[sl, :] = jnp.dot(kvb, wo_v[sl, :], preferred_element_type=F32).astype(BF)
            z = jnp.sum(z_acc[sl, :], axis=-1, keepdims=True)
            zb_v[sl, :] = jnp.where(mask, z, 0.0).astype(BF)

    wr = wr_ref[...].astype(F32)

    with jax.named_scope("phaseB"):
        @pl.loop(0, NB)
        def _(i):
            rows = pl.ds(pl.multiple_of(i * TM, TM), TM)
            pq = pq_v[rows, :]
            parts = []
            for g in range(G):
                pg = pq[:, g * 128:(g + 1) * 128]
                den = jnp.dot(pg, zb_v[pl.ds(g * 128, 128), :], preferred_element_type=F32) + 1e-6
                parts.append((pg.astype(F32) / den).astype(BF))
            a = jnp.concatenate(parts, axis=1)
            out = jnp.dot(a, m_v[...], preferred_element_type=F32)
            h = (x_v[rows, :].astype(F32) + out).astype(BF).astype(F32)
            hn = _ln(h).astype(BF)
            hnf = hn.astype(F32)
            r = jnp.sum(hnf * wr, axis=-1, keepdims=True).astype(BF).astype(F32)
            r_v[rows, :] = jnp.broadcast_to(r, (TM, 128))
            xn_v[rows, :] = hn
            x_v[rows, :] = (h + hnf).astype(BF)
            o_copy(i).start()

    with jax.named_scope("top2"):
        r = r_v[...]
        io = lax.broadcasted_iota(jnp.int32, (S, 128), 0)
        m1 = jnp.max(r)
        i1 = jnp.min(jnp.where(r == m1, io, S - 1))
        r2 = jnp.where(io == i1, -jnp.inf, r)
        m2 = jnp.max(r2)
        i2 = jnp.min(jnp.where(r2 == m2, io, S - 1))
        b1 = pl.multiple_of((i1 // 16) * 16, 16)
        b2 = pl.multiple_of((i2 // 16) * 16, 16)
        xs = jnp.concatenate([xn_v[pl.ds(b1, 16), :], xn_v[pl.ds(b2, 16), :]], axis=0)

    with jax.named_scope("ffn"):
        cg.wait()
        cu.wait()
        g_ = jnp.dot(xs, wg_v[...], preferred_element_type=F32)
        u_ = jnp.dot(xs, wu_v[...], preferred_element_type=F32)
        a = (g_ * jax.nn.sigmoid(g_) * u_).astype(BF)
        cd.wait()
        y = jnp.dot(a, wd_v[...], preferred_element_type=F32)

    with jax.named_scope("patch"):
        for i in range(NB):
            o_copy(i).wait()
        sub = lax.broadcasted_iota(jnp.int32, (16, D), 0)
        for (bb, ii, mm, yy, s) in ((b1, i1, m1, y[0:16], 0), (b2, i2, m2, y[16:32], 1)):
            sg = jax.nn.sigmoid(jnp.full((16, D), mm, F32))
            upd = jnp.where(sub == (ii - bb), yy * sg, 0.0)
            x_v[pl.ds(bb, 16), :] = (x_v[pl.ds(bb, 16), :].astype(F32) + upd).astype(BF)
            c = pltpu.make_async_copy(x_v.at[pl.ds(bb, 16)], out_hbm.at[pl.ds(bb, 16)], osem.at[NB + s])
            c.start()
            c.wait()


@jax.jit
def pallas_sequential_preLN__linear_attn_block__moe_arch_mod__prompt_kernel(
    A_x, A_wqkv, A_wo, B_x, B_w_r, B_w_gate, B_w_up, B_w_down):
    del B_x
    x = A_x.reshape(S, D)
    wr = B_w_r.reshape(1, D)
    anyspec = pl.BlockSpec(memory_space=pl.ANY)
    out = pl.pallas_call(
        _kernel,
        out_shape=jax.ShapeDtypeStruct((S, D), BF),
        in_specs=[anyspec, anyspec, anyspec, pl.BlockSpec(memory_space=pltpu.VMEM), anyspec, anyspec, anyspec],
        out_specs=anyspec,
        scratch_shapes=[
            pltpu.VMEM((S, D), BF), pltpu.VMEM((S, D), BF), pltpu.VMEM((S, D), BF),
            pltpu.VMEM((D, D), BF), pltpu.VMEM((D, D), BF), pltpu.VMEM((D, D), BF), pltpu.VMEM((D, D), BF),
            pltpu.VMEM((D, D), BF), pltpu.VMEM((D, D), BF), pltpu.VMEM((D, 128), BF),
            pltpu.VMEM((D, D), F32), pltpu.VMEM((D, 128), F32), pltpu.VMEM((S, 128), F32),
            pltpu.VMEM((D, F), BF), pltpu.VMEM((D, F), BF), pltpu.VMEM((F, D), BF),
            pltpu.SemaphoreType.DMA((NB,)), pltpu.SemaphoreType.DMA((7,)), pltpu.SemaphoreType.DMA((NB + 2,)),
        ],
        compiler_params=pltpu.CompilerParams(vmem_limit_bytes=110 * 1024 * 1024),
    )(x, A_wqkv, A_wo, wr, B_w_gate, B_w_up, B_w_down)
    return out.reshape(1, S, D)
```

```python
import jax
import numpy as np
import jax.numpy as jnp
from jax import lax
import jax.experimental.pallas as pl
import jax.experimental.pallas.tpu as pltpu

S, D, F, H, DH = 2048, 1024, 3584, 32, 32
TM = 512
TC = 256
CW = 32
B2 = [0, 512, 1024, 1536, 2048]
NT_ = S // TC
NB = S // TM
G = D // 128
FC = F // 128
BF = jnp.bfloat16
F32 = jnp.float32
NT = (((1,), (1,)), ((), ()))


def _phi(t):
    return jnp.where(t > 0, t + 1.0, jnp.exp(t)) + 1e-6


def _ln(x):
    m = jnp.mean(x, axis=-1, keepdims=True)
    c = x - m
    v = jnp.mean(c * c, axis=-1, keepdims=True)
    return c * lax.rsqrt(v + 1e-5)


def _kernel(z_ref, x_hbm, wqkv_hbm, wo_hbm, wr_ref, wg_hbm, wu_hbm, wd_hbm, out_hbm,
            x_v, xn_v, pq_v, wq_v, wk_v, wv_v, wkT_v, wo_v, m_v, zb_v, p_acc, z_acc,
            h_v, wg_v, wu_v, wd_v, xsem, qsem, wsem, osem):
    zero = z_ref[0]

    def tie(val, dep):
        if dep is None:
            return val
        t = pltpu.bitcast(dep, jnp.int32) & zero
        vi = pltpu.bitcast(val, jnp.int32)
        t = jnp.tile(t, (vi.shape[0] // 8, vi.shape[1] // 128))
        return pltpu.bitcast(vi | t, val.dtype)

    XB = [0, TC, 512, 1024, 2048]
    xc = [pltpu.make_async_copy(x_hbm.at[pl.ds(XB[i], XB[i + 1] - XB[i])], x_v.at[pl.ds(XB[i], XB[i + 1] - XB[i])],
                                xsem.at[i]) for i in range(4)]
    QC = 4
    qw = D // QC
    cq = [pltpu.make_async_copy(wqkv_hbm.at[:, pl.ds(c * qw, qw)], wq_v.at[:, pl.ds(c * qw, qw)], qsem.at[c])
          for c in range(QC)]
    ck = [pltpu.make_async_copy(wqkv_hbm.at[:, pl.ds(D + c * qw, qw)], wk_v.at[:, pl.ds(c * qw, qw)], qsem.at[QC + c])
          for c in range(QC)]
    cv = pltpu.make_async_copy(wqkv_hbm.at[:, pl.ds(2 * D, D)], wv_v, wsem.at[2])
    co = pltpu.make_async_copy(wo_hbm, wo_v, wsem.at[3])
    cg = [pltpu.make_async_copy(wg_hbm.at[:, pl.ds(c * 128, 128)], wg_v.at[c], wsem.at[4]) for c in range(FC)]
    cu = [pltpu.make_async_copy(wu_hbm.at[:, pl.ds(c * 128, 128)], wu_v.at[c], wsem.at[5]) for c in range(FC)]
    cd = [pltpu.make_async_copy(wd_hbm.at[:, pl.ds(c * 128, 128)], wd_v.at[c], wsem.at[6]) for c in range(G)]

    xc[0].start()
    for c in cq:
        c.start()

    def R(t):
        return pl.ds(t * TC, TC)

    def ln_chunk(t, dep, c=0, n=1):
        if t * TC in XB and c == 0:
            xc[XB.index(t * TC)].wait()
        rows = pl.ds(t * TC + c * (TC // n), TC // n)
        x = x_v[rows, :].astype(F32)
        xn = _ln(tie(x, dep))
        xn_v[rows, :] = xn.astype(BF)
        return xn[-8:, -128:]

    def q_chunk(t, dep, c=0, n=1):
        cols = pl.ds(c * (D // n), D // n)
        q = jnp.dot(tie(xn_v[R(t), :], dep), wq_v[:, cols], preferred_element_type=F32)
        pq_v[R(t), cols] = _phi(q).astype(BF)
        return q[:8, :128]

    def kp_chunk(t, dep):
        xn = tie(xn_v[R(t), :], dep)
        kT = lax.dot_general(wkT_v[...], xn, NT, preferred_element_type=F32)
        pk = _phi(kT)
        zs = pk[:, 0:128]
        for j in range(1, TC // 128):
            zs = zs + pk[:, j * 128:(j + 1) * 128]
        pp = jnp.dot(pk.astype(BF), xn, preferred_element_type=F32)
        if t == 0:
            z_acc[...] = zs
            p_acc[...] = pp
        else:
            z_acc[...] += zs
            p_acc[...] += pp
        return kT[:8, :128]

    rr = lax.broadcasted_iota(jnp.int32, (128, 128), 0) // DH
    cc = lax.broadcasted_iota(jnp.int32, (128, 128), 1) // DH
    mask = rr == cc

    def mid_chunk(g):
        sl = pl.ds(g * 128, 128)
        kv = jnp.dot(p_acc[sl, :].astype(BF), wv_v[:, sl], preferred_element_type=F32)
        kvb = jnp.where(mask, kv, 0.0).astype(BF)
        m_v[sl, :] = jnp.dot(kvb, wo_v[sl, :], preferred_element_type=F32).astype(BF)
        z = jnp.sum(z_acc[sl, :], axis=-1, keepdims=True)
        zb_v[sl, :] = jnp.where(mask, z, 0.0).astype(BF)

    ln_chunk(0, None)
    for c in range(QC):
        cq[c].wait()
        if c == 1:
            xc[1].start()
        if c == 2:
            for k_ in ck:
                k_.start()
        dq = q_chunk(0, None, c, QC)
    dl = ln_chunk(1, None)
    xc[2].start()
    for k_ in ck:
        k_.wait()
    dq = q_chunk(1, dl)
    for g in range(G):
        wkT_v[pl.ds(g * 128, 128), :] = wk_v[:, pl.ds(g * 128, 128)].T
    xc[3].start()
    ln_chunk(2, None)
    cv.start()
    co.start()
    LQ = 512 // TC
    dl = None
    for t in range(NT_):
        dq = kp_chunk(t, dl)
        if t == 1:
            for c in cg + cu + cd:
                c.start()
        if t + 2 < NT_ - LQ:
            dl = None
            for c in range(4):
                dn = ln_chunk(t + 3, dq, c, 4) if t + 3 < NT_ else None
                dq = q_chunk(t + 2, dl, c, 4)
                dl = dn
            if t + 2 == NT_ - LQ - 1:
                for tt in range(t + 4, NT_):
                    dl = ln_chunk(tt, dq)
        else:
            dl = None
    cv.wait()
    co.wait()
    for k in range(LQ):
        q_chunk(NT_ - LQ + k, None)
        for g in range(k * G // LQ, (k + 1) * G // LQ):
            mid_chunk(g)

    wr = wr_ref[...].astype(F32).reshape(1, D)
    lane = lax.broadcasted_iota(jnp.int32, (8, 128), 1)
    rv = [jnp.full((8, 128), -jnp.inf, F32) for _ in range(S // 1024)]

    def a_chunk(i, g):
        rows = pl.ds(B2[i], B2[i + 1] - B2[i])
        sl = pl.ds(g * 128, 128)
        pg = pq_v[rows, sl]
        den = jnp.dot(pg, zb_v[sl, :], preferred_element_type=F32) + 1e-6
        pq_v[rows, sl] = (pg.astype(F32) * pl.reciprocal(den, approx=True)).astype(BF)

    def b_chunk(i, j, dep):
        rows = pl.ds(B2[i], B2[i + 1] - B2[i])
        sl = pl.ds(j * 128, 128)
        out = jnp.dot(pq_v[rows, :], tie(m_v[:, sl], dep), preferred_element_type=F32)
        h_v[rows, sl] = x_v[rows, sl].astype(F32) + out
        return out[:8, :]

    def c_chunk(i, j, dep):
        w = (B2[i + 1] - B2[i]) // G
        if i == len(B2) - 2:
            return c_sub(B2[i] + j * w, w, None)
        for u in range(w // CW):
            dep = c_sub(B2[i] + j * w + u * CW, CW, dep)
        return dep

    def c_sub(r0, w, dep):
        rows = pl.ds(r0, w)
        h = tie(h_v[rows, :], dep)
        hnf = _ln(h)
        hn = hnf.astype(BF)
        r = jnp.sum(hnf * wr, axis=-1, keepdims=True).astype(BF).astype(F32)
        for k in range(w // 8):
            gi = r0 // 8 + k
            rv[gi // 128] = jnp.where(lane == (gi % 128), r[k * 8:(k + 1) * 8], rv[gi // 128])
        xn_v[rows, :] = hn
        x_v[rows, :] = (h + hnf).astype(BF)
        return rv[gi // 128]

    N2 = len(B2) - 1
    for g in range(G):
        a_chunk(0, g)
    db = dc = dc2 = None
    for i in range(N2 + 1):
        for j in range(G):
            dcn = c_chunk(i - 1, j, db) if i >= 1 else None
            db = b_chunk(i, j, dc) if i < N2 else None
            dc2, dc = dc, dcn
            if i + 1 < N2:
                a_chunk(i + 1, j)
        if i >= 1:
            rws = pl.ds(B2[i - 1], B2[i] - B2[i - 1])
            pltpu.make_async_copy(x_v.at[rws], out_hbm.at[rws], osem.at[0]).start()

    tok = [lax.broadcasted_iota(jnp.int32, (8, 128), 0) + 8 * (lane + 128 * k) for k in range(len(rv))]
    r = jnp.concatenate(rv, axis=1)
    io = jnp.concatenate(tok, axis=1)
    m1 = jnp.max(r)
    i1 = jnp.min(jnp.where(r == m1, io, S - 1))
    r2 = jnp.where(io == i1, -jnp.inf, r)
    m2 = jnp.max(r2)
    i2 = jnp.min(jnp.where(r2 == m2, io, S - 1))
    b1 = pl.multiple_of((i1 // 16) * 16, 16)
    b2 = pl.multiple_of((i2 // 16) * 16, 16)
    sub = lax.broadcasted_iota(jnp.int32, (16, D), 0)
    row1 = jnp.sum(jnp.where(sub == i1 - b1, xn_v[pl.ds(b1, 16), :].astype(F32), 0.0), axis=0, keepdims=True)
    row2 = jnp.sum(jnp.where(sub == i2 - b2, xn_v[pl.ds(b2, 16), :].astype(F32), 0.0), axis=0, keepdims=True)
    xs = jnp.where(sub == 0, row1, row2).astype(BF)

    pltpu.make_async_copy(wg_v, wg_v, wsem.at[4]).wait()
    pltpu.make_async_copy(wu_v, wu_v, wsem.at[5]).wait()
    acts = []
    for c in range(FC):
        g_ = jnp.dot(xs, wg_v[c], preferred_element_type=F32)
        u_ = jnp.dot(xs, wu_v[c], preferred_element_type=F32)
        acts.append((g_ * jax.nn.sigmoid(g_) * u_).astype(BF))
    a = jnp.concatenate(acts, axis=1)
    pltpu.make_async_copy(wd_v, wd_v, wsem.at[6]).wait()
    y = jnp.concatenate([jnp.dot(a, wd_v[c], preferred_element_type=F32) for c in range(G)], axis=1)

    pltpu.make_async_copy(x_v, out_hbm, osem.at[0]).wait()
    for (bb, ii, mm, s) in ((b1, i1, m1, 0), (b2, i2, m2, 1)):
        sg = jax.nn.sigmoid(jnp.full((16, D), mm, F32))
        upd = jnp.where(sub == (ii - bb), y[s:s + 1] * sg, 0.0)
        x_v[pl.ds(bb, 16), :] = (x_v[pl.ds(bb, 16), :].astype(F32) + upd).astype(BF)
    p1 = pltpu.make_async_copy(x_v.at[pl.ds(b1, 16)], out_hbm.at[pl.ds(b1, 16)], osem.at[1])
    p2 = pltpu.make_async_copy(x_v.at[pl.ds(b2, 16)], out_hbm.at[pl.ds(b2, 16)], osem.at[2])
    p1.start()

    @pl.when(b1 != b2)
    def _():
        p2.start()
        p2.wait()

    p1.wait()


@jax.jit
def pallas_sequential_preLN__linear_attn_block__moe_arch_mod__prompt_kernel(
    A_x, A_wqkv, A_wo, B_x, B_w_r, B_w_gate, B_w_up, B_w_down):
    del B_x
    x = A_x.reshape(S, D)
    wr = B_w_r
    anyspec = pl.BlockSpec(memory_space=pl.ANY)
    out = pl.pallas_call(
        _kernel,
        out_shape=jax.ShapeDtypeStruct((S, D), BF),
        in_specs=[pl.BlockSpec(memory_space=pltpu.SMEM), anyspec, anyspec, anyspec, pl.BlockSpec(memory_space=pltpu.VMEM), anyspec, anyspec, anyspec],
        out_specs=anyspec, grid=(1,),
        scratch_shapes=[
            pltpu.VMEM((S, D), BF), pltpu.VMEM((S, D), BF), pltpu.VMEM((S, D), BF),
            pltpu.VMEM((D, D), BF), pltpu.VMEM((D, D), BF), pltpu.VMEM((D, D), BF), pltpu.VMEM((D, D), BF),
            pltpu.VMEM((D, D), BF), pltpu.VMEM((D, D), BF), pltpu.VMEM((D, 128), BF),
            pltpu.VMEM((D, D), F32), pltpu.VMEM((D, 128), F32), pltpu.VMEM((S, D), F32),
            pltpu.VMEM((FC, D, 128), BF), pltpu.VMEM((FC, D, 128), BF), pltpu.VMEM((G, F, 128), BF),
            pltpu.SemaphoreType.DMA((4,)), pltpu.SemaphoreType.DMA((8,)), pltpu.SemaphoreType.DMA((7,)),
            pltpu.SemaphoreType.DMA((NB + 2,)),
        ],
        compiler_params=pltpu.CompilerParams(vmem_limit_bytes=110 * 1024 * 1024),
    )(np.zeros((1,), np.int32), x, A_wqkv, A_wo, wr, B_w_gate, B_w_up, B_w_down)
    return out.reshape(1, S, D)
```

```python
import jax
import numpy as np
import jax.numpy as jnp
from jax import lax
import jax.experimental.pallas as pl
import jax.experimental.pallas.tpu as pltpu

S, D, F, H, DH = 2048, 1024, 3584, 32, 32
TM = 512
TC = 256
CW = 32
B2 = [0, 512, 1024, 1536, 2048]
NT_ = S // TC
NB = S // TM
G = D // 128
FC = F // 128
BF = jnp.bfloat16
F32 = jnp.float32
NT = (((1,), (1,)), ((), ()))


def _phi(t):
    return jnp.where(t > 0, t + 1.0, jnp.exp(t)) + 1e-6


def _ln(x):
    m = jnp.mean(x, axis=-1, keepdims=True)
    c = x - m
    v = jnp.mean(c * c, axis=-1, keepdims=True)
    return c * lax.rsqrt(v + 1e-5)


def _kernel(z_ref, x_hbm, wqkv_hbm, wo_hbm, wr_ref, wg_hbm, wu_hbm, wd_hbm, out_hbm,
            x_v, xn_v, pq_v, wq_v, wk_v, wv_v, wkT_v, wo_v, m_v, zb_v, p_acc, z_acc,
            h_v, wg_v, wu_v, wd_v, xsem, qsem, wsem, osem):
    zero = z_ref[0]

    def tie(val, dep):
        if dep is None:
            return val
        t = pltpu.bitcast(dep, jnp.int32) & zero
        vi = pltpu.bitcast(val, jnp.int32)
        t = jnp.tile(t, (vi.shape[0] // 8, vi.shape[1] // 128))
        return pltpu.bitcast(vi | t, val.dtype)

    XB = [0, TC, 512, 1024, 2048]
    xc = [pltpu.make_async_copy(x_hbm.at[pl.ds(XB[i], XB[i + 1] - XB[i])], x_v.at[pl.ds(XB[i], XB[i + 1] - XB[i])],
                                xsem.at[i]) for i in range(4)]
    QC = 4
    qw = D // QC
    cq = [pltpu.make_async_copy(wqkv_hbm.at[:, pl.ds(c * qw, qw)], wq_v.at[:, pl.ds(c * qw, qw)], qsem.at[c])
          for c in range(QC)]
    ck = [pltpu.make_async_copy(wqkv_hbm.at[:, pl.ds(D, D)], wk_v, qsem.at[QC])]
    cv = pltpu.make_async_copy(wqkv_hbm.at[:, pl.ds(2 * D, D)], wv_v, wsem.at[2])
    co = pltpu.make_async_copy(wo_hbm, wo_v, wsem.at[3])
    cg = [pltpu.make_async_copy(wg_hbm.at[:, pl.ds(c * 128, 128)], wg_v.at[c], wsem.at[4]) for c in range(FC)]
    cu = [pltpu.make_async_copy(wu_hbm.at[:, pl.ds(c * 128, 128)], wu_v.at[c], wsem.at[5]) for c in range(FC)]
    cd = [pltpu.make_async_copy(wd_hbm.at[:, pl.ds(c * 128, 128)], wd_v.at[c], wsem.at[6]) for c in range(G)]

    xc[0].start()
    cq[0].start()

    def R(t):
        return pl.ds(t * TC, TC)

    def ln_chunk(t, dep, c=0, n=1):
        if t * TC in XB and c == 0 and t > 0:
            xc[XB.index(t * TC)].wait()
        rows = pl.ds(t * TC + c * (TC // n), TC // n)
        x = x_v[rows, :].astype(F32)
        xn = _ln(tie(x, dep))
        xn_v[rows, :] = xn.astype(BF)
        return xn[-8:, -128:]

    def q_chunk(t, dep, c=0, n=1):
        cols = pl.ds(c * (D // n), D // n)
        q = jnp.dot(tie(xn_v[R(t), :], dep), wq_v[:, cols], preferred_element_type=F32)
        pq_v[R(t), cols] = _phi(q).astype(BF)
        return q[:8, :128]

    def kp_chunk(t, dep):
        xn = tie(xn_v[R(t), :], dep)
        kT = lax.dot_general(wkT_v[...], xn, NT, preferred_element_type=F32)
        pk = _phi(kT)
        zs = pk[:, 0:128]
        for j in range(1, TC // 128):
            zs = zs + pk[:, j * 128:(j + 1) * 128]
        pp = jnp.dot(pk.astype(BF), xn, preferred_element_type=F32)
        if t == 0:
            z_acc[...] = zs
            p_acc[...] = pp
        else:
            z_acc[...] += zs
            p_acc[...] += pp
        return kT[:8, :128]

    rr = lax.broadcasted_iota(jnp.int32, (128, 128), 0) // DH
    cc = lax.broadcasted_iota(jnp.int32, (128, 128), 1) // DH
    mask = rr == cc

    def mid_chunk(g):
        sl = pl.ds(g * 128, 128)
        kv = jnp.dot(p_acc[sl, :].astype(BF), wv_v[:, sl], preferred_element_type=F32)
        kvb = jnp.where(mask, kv, 0.0).astype(BF)
        m_v[sl, :] = jnp.dot(kvb, wo_v[sl, :], preferred_element_type=F32).astype(BF)
        z = jnp.sum(z_acc[sl, :], axis=-1, keepdims=True)
        zb_v[sl, :] = jnp.where(mask, z, 0.0).astype(BF)

    xc[0].wait()
    for c in cq[1:]:
        c.start()
    ln_chunk(0, None)
    for c in range(QC):
        cq[c].wait()
        if c == 0:
            xc[1].start()
        if c == 1:
            for k_ in ck:
                k_.start()
        dq = q_chunk(0, None, c, QC)
    dl = ln_chunk(1, None)
    xc[2].start()
    q_chunk(1, dl)
    for k_ in ck:
        k_.wait()
    dl = ln_chunk(2, None)
    dq = q_chunk(2, dl)
    for g in range(G):
        wkT_v[pl.ds(g * 128, 128), :] = wk_v[:, pl.ds(g * 128, 128)].T
    xc[3].start()
    ln_chunk(3, None)
    cv.start()
    co.start()
    LQ = 512 // TC
    dl = None
    for t in range(NT_):
        dq = kp_chunk(t, dl)
        if t == 1:
            for c in cg + cu + cd:
                c.start()
        if t + 3 < NT_ - LQ:
            dl = None
            for c in range(4):
                dn = ln_chunk(t + 4, dq, c, 4) if t + 4 < NT_ else None
                dq = q_chunk(t + 3, dl, c, 4)
                dl = dn
            if t + 3 == NT_ - LQ - 1:
                for tt in range(t + 5, NT_):
                    dl = ln_chunk(tt, dq)
        else:
            dl = None
    cv.wait()
    co.wait()
    for k in range(LQ):
        q_chunk(NT_ - LQ + k, None)
        for g in range(k * G // LQ, (k + 1) * G // LQ):
            mid_chunk(g)

    wr = wr_ref[...].astype(F32).reshape(1, D)
    lane = lax.broadcasted_iota(jnp.int32, (8, 128), 1)
    rv = [jnp.full((8, 128), -jnp.inf, F32) for _ in range(S // 1024)]

    def a_chunk(i, g):
        rows = pl.ds(B2[i], B2[i + 1] - B2[i])
        sl = pl.ds(g * 128, 128)
        pg = pq_v[rows, sl]
        den = jnp.dot(pg, zb_v[sl, :], preferred_element_type=F32) + 1e-6
        pq_v[rows, sl] = (pg.astype(F32) * pl.reciprocal(den, approx=True)).astype(BF)

    def b_chunk(i, j, dep):
        rows = pl.ds(B2[i], B2[i + 1] - B2[i])
        sl = pl.ds(j * 128, 128)
        out = jnp.dot(pq_v[rows, :], tie(m_v[:, sl], dep), preferred_element_type=F32)
        h_v[rows, sl] = x_v[rows, sl].astype(F32) + out
        return out[:8, :]

    def c_chunk(i, j, dep):
        w = (B2[i + 1] - B2[i]) // G
        if i == len(B2) - 2:
            return c_sub(B2[i] + j * w, w, None)
        for u in range(w // CW):
            dep = c_sub(B2[i] + j * w + u * CW, CW, dep)
        return dep

    def c_sub(r0, w, dep):
        rows = pl.ds(r0, w)
        h = tie(h_v[rows, :], dep)
        hnf = _ln(h)
        hn = hnf.astype(BF)
        r = jnp.sum(hnf * wr, axis=-1, keepdims=True).astype(BF).astype(F32)
        for k in range(w // 8):
            gi = r0 // 8 + k
            rv[gi // 128] = jnp.where(lane == (gi % 128), r[k * 8:(k + 1) * 8], rv[gi // 128])
        xn_v[rows, :] = hn
        x_v[rows, :] = (h + hnf).astype(BF)
        return rv[gi // 128]

    N2 = len(B2) - 1
    for g in range(G):
        a_chunk(0, g)
    db = dc = dc2 = None
    for i in range(N2 + 1):
        for j in range(G):
            dcn = c_chunk(i - 1, j, db) if i >= 1 else None
            db = b_chunk(i, j, dc) if i < N2 else None
            dc2, dc = dc, dcn
            if i + 1 < N2:
                a_chunk(i + 1, j)
        if i >= 1:
            rws = pl.ds(B2[i - 1], B2[i] - B2[i - 1])
            pltpu.make_async_copy(x_v.at[rws], out_hbm.at[rws], osem.at[0]).start()

    tok = [lax.broadcasted_iota(jnp.int32, (8, 128), 0) + 8 * (lane + 128 * k) for k in range(len(rv))]
    r = jnp.concatenate(rv, axis=1)
    io = jnp.concatenate(tok, axis=1)
    m1 = jnp.max(r)
    i1 = jnp.min(jnp.where(r == m1, io, S - 1))
    r2 = jnp.where(io == i1, -jnp.inf, r)
    m2 = jnp.max(r2)
    i2 = jnp.min(jnp.where(r2 == m2, io, S - 1))
    b1 = pl.multiple_of((i1 // 16) * 16, 16)
    b2 = pl.multiple_of((i2 // 16) * 16, 16)
    sub = lax.broadcasted_iota(jnp.int32, (16, D), 0)
    row1 = jnp.sum(jnp.where(sub == i1 - b1, xn_v[pl.ds(b1, 16), :].astype(F32), 0.0), axis=0, keepdims=True)
    row2 = jnp.sum(jnp.where(sub == i2 - b2, xn_v[pl.ds(b2, 16), :].astype(F32), 0.0), axis=0, keepdims=True)
    xs = jnp.where(sub == 0, row1, row2).astype(BF)

    pltpu.make_async_copy(wg_v, wg_v, wsem.at[4]).wait()
    pltpu.make_async_copy(wu_v, wu_v, wsem.at[5]).wait()
    acts = []
    for c in range(FC):
        g_ = jnp.dot(xs, wg_v[c], preferred_element_type=F32)
        u_ = jnp.dot(xs, wu_v[c], preferred_element_type=F32)
        acts.append((g_ * jax.nn.sigmoid(g_) * u_).astype(BF))
    a = jnp.concatenate(acts, axis=1)
    pltpu.make_async_copy(wd_v, wd_v, wsem.at[6]).wait()
    y = jnp.concatenate([jnp.dot(a, wd_v[c], preferred_element_type=F32) for c in range(G)], axis=1)

    pltpu.make_async_copy(x_v, out_hbm, osem.at[0]).wait()
    for (bb, ii, mm, s) in ((b1, i1, m1, 0), (b2, i2, m2, 1)):
        sg = jax.nn.sigmoid(jnp.full((16, D), mm, F32))
        upd = jnp.where(sub == (ii - bb), y[s:s + 1] * sg, 0.0)
        x_v[pl.ds(bb, 16), :] = (x_v[pl.ds(bb, 16), :].astype(F32) + upd).astype(BF)
    p1 = pltpu.make_async_copy(x_v.at[pl.ds(b1, 16)], out_hbm.at[pl.ds(b1, 16)], osem.at[1])
    p2 = pltpu.make_async_copy(x_v.at[pl.ds(b2, 16)], out_hbm.at[pl.ds(b2, 16)], osem.at[2])
    p1.start()

    @pl.when(b1 != b2)
    def _():
        p2.start()
        p2.wait()

    p1.wait()


@jax.jit
def pallas_sequential_preLN__linear_attn_block__moe_arch_mod__prompt_kernel(
    A_x, A_wqkv, A_wo, B_x, B_w_r, B_w_gate, B_w_up, B_w_down):
    del B_x
    x = A_x.reshape(S, D)
    wr = B_w_r
    anyspec = pl.BlockSpec(memory_space=pl.ANY)
    out = pl.pallas_call(
        _kernel,
        out_shape=jax.ShapeDtypeStruct((S, D), BF),
        in_specs=[pl.BlockSpec(memory_space=pltpu.SMEM), anyspec, anyspec, anyspec, pl.BlockSpec(memory_space=pltpu.VMEM), anyspec, anyspec, anyspec],
        out_specs=anyspec, grid=(1,),
        scratch_shapes=[
            pltpu.VMEM((S, D), BF), pltpu.VMEM((S, D), BF), pltpu.VMEM((S, D), BF),
            pltpu.VMEM((D, D), BF), pltpu.VMEM((D, D), BF), pltpu.VMEM((D, D), BF), pltpu.VMEM((D, D), BF),
            pltpu.VMEM((D, D), BF), pltpu.VMEM((D, D), BF), pltpu.VMEM((D, 128), BF),
            pltpu.VMEM((D, D), F32), pltpu.VMEM((D, 128), F32), pltpu.VMEM((S, D), F32),
            pltpu.VMEM((FC, D, 128), BF), pltpu.VMEM((FC, D, 128), BF), pltpu.VMEM((G, F, 128), BF),
            pltpu.SemaphoreType.DMA((4,)), pltpu.SemaphoreType.DMA((8,)), pltpu.SemaphoreType.DMA((7,)),
            pltpu.SemaphoreType.DMA((NB + 2,)),
        ],
        compiler_params=pltpu.CompilerParams(vmem_limit_bytes=110 * 1024 * 1024),
    )(np.zeros((1,), np.int32), x, A_wqkv, A_wo, wr, B_w_gate, B_w_up, B_w_down)
    return out.reshape(1, S, D)
```
